```python
import os as _os
_os.environ.setdefault("JAX_PLATFORMS", "cpu")
import jax
import jax.numpy as jnp

def _softmax(x, axis=-1):
    return jax.nn.softmax(x, axis=axis)
def _gelu(x):
    return jax.nn.gelu(x, approximate=True)
def _silu(x):
    return jax.nn.silu(x)
def _sigmoid(x):
    return jax.nn.sigmoid(x)
def _layernorm(x, axis=-1, eps=1e-5):
    m = jnp.mean(x, axis=axis, keepdims=True)
    v = jnp.var(x, axis=axis, keepdims=True)
    return (x - m) / jnp.sqrt(v + eps)
def _scatter_add(tgt, idx, src, axis=0):
    return tgt.at[idx].add(src)
def _segment_sum(src, seg, n):
    return jax.ops.segment_sum(src, seg, n)
class _Rng:
    def __init__(self, key):
        self._k = key
    def _next(self):
        self._k, sub = jax.random.split(self._k)
        return sub
    def normal(self, shape):
        return jax.random.normal(self._next(), shape, dtype=jnp.bfloat16)
    def randint(self, lo, hi, shape):
        return jax.random.randint(self._next(), shape, lo, hi, dtype=jnp.int32)
    def uniform(self, shape, lo=0.0, hi=1.0):
        return jax.random.uniform(self._next(), shape, jnp.bfloat16, lo, hi)
    def permutation(self, n):
        return jax.random.permutation(self._next(), n)


kernel_name = 'interleave_layers__linear_kernel_hedgehog__dense_activation_silu__prompt'

def setup_inputs():
    _rng = _Rng(jax.random.key(int.from_bytes(__import__("os").urandom(4), "little")))
    _w = (lambda a: (lambda t: t.astype(jnp.bfloat16) if jnp.issubdtype(t.dtype, jnp.floating) else t)(jnp.asarray(a)))
    def _A_setup():
        B, S, D, H = 1, 2048, 640, 32
        Dh = D // H
        return {
            "x": _w((lambda *s: _rng.normal(s) * 0.05)(B, S, D)),
            "wqkv": _w((lambda *s: _rng.normal(s) * 0.4)(D, 3 * D)),
            "w_phi": _w((lambda *s: _rng.normal(s) * 0.4)(H, Dh, Dh) * (Dh ** -0.5)),
            "wo": _w((lambda *s: _rng.normal(s) * 0.05)(D, D)),
        }
    _A_in = _A_setup()

    def _B_setup():
        B, S, D, F = 1, 2048, 640, 1728
        return {
            "x": _w((lambda *s: _rng.normal(s) * 0.05)(B, S, D)),
            "w1": _w((lambda *s: _rng.normal(s) * 1.6)(D, F) * (D ** -0.5)),
            "w2": _w((lambda *s: _rng.normal(s) * 1.6)(F, D) * (F ** -0.5)),
        }
    _B_in = _B_setup()

    return {
        "A_x": _A_in["x"],
        "A_wqkv": _A_in["wqkv"],
        "A_w_phi": _A_in["w_phi"],
        "A_wo": _A_in["wo"],
        "B_x": _B_in["x"],
        "B_w1": _B_in["w1"],
        "B_w2": _B_in["w2"],
    }

def reference(A_x, A_wqkv, A_w_phi, A_wo, B_x, B_w1, B_w2):
    def _A_ref(x, wqkv, w_phi, wo):
        B, S, D = x.shape
        H = 32; Dh = D // H
        qkv = (lambda x, *d: x.transpose(*d))((x @ wqkv).reshape(B, S, 3, H, Dh), 2, 0, 3, 1, 4)
        q, k, v = qkv[0], qkv[1], qkv[2]
        pq = jnp.einsum("bhsd,hdf->bhsf", q, w_phi)
        pk = jnp.einsum("bhsd,hdf->bhsf", k, w_phi)
        phi_q = jnp.concatenate([_softmax(pq, axis=-1), _softmax(-pq, axis=-1)], axis=-1)
        phi_k = jnp.concatenate([_softmax(pk, axis=-1), _softmax(-pk, axis=-1)], axis=-1)
        kv = jnp.einsum("bhsf,bhsd->bhfd", phi_k, v)
        z  = jnp.einsum("bhsf->bhf", phi_k)
        num = jnp.einsum("bhqf,bhfd->bhqd", phi_q, kv)
        den = jnp.einsum("bhqf,bhf->bhq", phi_q, z)[..., None] + 1e-6
        o = num / den
        return (lambda x, *d: x.transpose(*d))(o, 0, 2, 1, 3).reshape(B, S, D) @ wo

    def _B_ref(x, w1, w2):
        h = jnp.einsum("bsd,df->bsf", x, w1)
        h = _silu(h)
        out = jnp.einsum("bsf,fd->bsd", h, w2)
        return out

    x = A_x
    x = x + _A_ref(_layernorm(x, axis=-1), A_wqkv, A_w_phi, A_wo)
    x = x + _B_ref(_layernorm(x, axis=-1), B_w1, B_w2)
    x = x + _A_ref(_layernorm(x, axis=-1), A_wqkv, A_w_phi, A_wo)
    x = x + _B_ref(_layernorm(x, axis=-1), B_w1, B_w2)
    return x
```

```python
import functools
import numpy as np
import jax
import jax.numpy as jnp
from jax import lax
import jax.experimental.pallas as pl
import jax.experimental.pallas.tpu as pltpu

S, D, F, H, DH = 2048, 640, 1728, 32, 20
NP = H // 2
PR = 2 * DH
LOG2E = 1.4426950408889634
f32, bf16 = jnp.float32, jnp.bfloat16
NN = (((1,), (0,)), ((), ()))
NT = (((1,), (1,)), ((), ()))
def _win(kt):
    lo = ((128 * kt) // PR) * PR
    hi = -((-128 * (kt + 1)) // PR) * PR
    lo = (lo // 16) * 16
    hi = min(-((-hi) // 16) * 16, D)
    return lo, hi


def _dot(a, b, dims=NN):
    return lax.dot_general(a, b, dims, preferred_element_type=f32)


def _ln(x):
    m = jnp.sum(x, axis=0, keepdims=True) * (1.0 / D)
    d = x - m
    v = jnp.sum(d * d, axis=0, keepdims=True) * (1.0 / D)
    return (d * lax.rsqrt(v + 1e-5)).astype(bf16)


def _par_reduce(v, op):
    v = op(v, pltpu.roll(v, 4, 0))
    return op(v, pltpu.roll(v, 2, 0))


def _tree(op, xs):
    r = xs[0]
    for v in xs[1:]:
        r = op(r, v)
    return r


def _phi(s):
    sl = [s[8 * i:8 * i + 8] for i in range(5)]
    mx = _par_reduce(_tree(jnp.maximum, sl), jnp.maximum)
    mn = _par_reduce(_tree(jnp.minimum, sl), jnp.minimum)
    ep = [jnp.exp2(v - mx) for v in sl]
    en = [jnp.exp2(mn - v) for v in sl]
    rp = 1.0 / _par_reduce(_tree(jnp.add, ep), jnp.add)
    rn = 1.0 / _par_reduce(_tree(jnp.add, en), jnp.add)
    return jnp.concatenate([v * rp for v in ep] + [v * rn for v in en], axis=0).astype(bf16)


def make(T=256, NI=2, RB=160):
    NC = S // T
    NB = NC // NI

    def kernel(x_hbm, wqkv_hbm, wphi_hbm, wo_hbm, w1_hbm, w2_hbm, o_hbm,
               xin, wqkv_v, wphi_v, wo_v, w1_v, w2_v,
               wqT, wkvT, woT, w1T, w2T, xT, xnT, macc, kvb, scr, outv, sems, osems):
        cps = [pltpu.make_async_copy(wphi_hbm, wphi_v, sems.at[0]),
               pltpu.make_async_copy(wqkv_hbm, wqkv_v, sems.at[1]),
               pltpu.make_async_copy(x_hbm, xin, sems.at[2]),
               pltpu.make_async_copy(wo_hbm, wo_v, sems.at[3]),
               pltpu.make_async_copy(w1_hbm, w1_v, sems.at[4]),
               pltpu.make_async_copy(w2_hbm, w2_v, sems.at[5])]
        for c in cps:
            c.start()
        macc[...] = jnp.zeros(macc.shape, f32)
        cps[0].wait()
        for h in range(H):
            scr[DH * h:DH * h + DH, :] = wphi_v[h].astype(f32)
        cps[1].wait()
        polita = []
        for kt in range(5):
            lo, hi = _win(kt)
            wl = hi - lo
            r = lax.broadcasted_iota(jnp.int32, (wl, DH), 0) + lo
            fcol = lax.broadcasted_iota(jnp.int32, (wl, DH), 1)
            p = ((r.astype(f32) + 0.5) * (1.0 / PR)).astype(jnp.int32)
            et = jnp.where(((r - p * PR) >> 1) == fcol, 1.0, 0.0).astype(bf16)
            bd = _dot(et, scr[128 * kt:128 * kt + 128, :].astype(bf16), NT)
            r2 = lax.broadcasted_iota(jnp.int32, (wl, 128), 0) + lo
            c2 = lax.broadcasted_iota(jnp.int32, (wl, 128), 1) + 128 * kt
            pr2 = ((r2.astype(f32) + 0.5) * (1.0 / PR)).astype(jnp.int32)
            hc2 = ((c2.astype(f32) + 0.5) * (1.0 / DH)).astype(jnp.int32)
            ok = (pr2 * 2 + (r2 & 1)) == hc2
            polita.append(jnp.where(ok, bd, 0.0).astype(bf16))
        for wsel, dst, off in ((1, wkvT, 0), (0, wqT, 0)):
            parts = []
            for kt in range(5):
                c0 = D * wsel + 128 * kt
                parts.append(_dot(polita[kt], wqkv_v[:, c0:c0 + 128], NT))
            for b in range(D // 16):
                acc = None
                for kt in range(5):
                    lo, hi = _win(kt)
                    if lo <= 16 * b < hi:
                        v = parts[kt][16 * b - lo:16 * b - lo + 16]
                        acc = v if acc is None else acc + v
                dst[off + 16 * b:off + 16 * b + 16, :] = (acc * LOG2E).astype(bf16)
        for kt in range(5):
            c0 = 2 * D + 128 * kt
            wkvT[D + 128 * kt:D + 128 * kt + 128, :] = wqkv_v[:, c0:c0 + 128].T

        ones8 = jnp.ones((8, T), f32)

        def stage_a(c, x):
            xn = _ln(x)
            xnT[c] = xn
            yield
            for r0 in range(0, D, RB):
                pk = _dot(wkvT[r0:r0 + RB, :], xn)
                vv = _dot(wkvT[D + r0:D + r0 + RB, :], xn)
                for j in range(RB // PR):
                    p = r0 // PR + j
                    ph = _phi(pk[PR * j:PR * j + PR])
                    vt = jnp.concatenate([vv[PR * j:PR * j + PR], ones8], axis=0).astype(bf16)
                    macc[p] += _dot(vt, ph, NT)
                yield

        def finalize():
            r = lax.broadcasted_iota(jnp.int32, (48, 2 * PR), 0)
            cc = lax.broadcasted_iota(jnp.int32, (48, 2 * PR), 1)
            hsel = jnp.where(r < 40, jnp.where(r >= DH, 1, 0), jnp.where(r >= 44, 1, 0))
            ok = hsel == (cc & 1)
            for p in range(NP):
                kvb[p] = jnp.where(ok, macc[p], 0.0).astype(bf16)
            macc[...] = jnp.zeros(macc.shape, f32)

        low4 = lax.broadcasted_iota(jnp.int32, (8, T), 0) < 4

        def stage_bc(c):
            xn = xnT[c]
            os_ = []
            for r0 in range(0, D, RB):
                pq = _dot(wqT[r0:r0 + RB, :], xn)
                for j in range(RB // PR):
                    p = r0 // PR + j
                    ph = _phi(pq[PR * j:PR * j + PR])
                    nd = _dot(kvb[p], ph)
                    rm = 1.0 / (nd[40:48] + 1e-6)
                    rr = pltpu.roll(rm, 4, 0)
                    ra = jnp.where(low4, rm, rr)
                    rb = jnp.where(low4, rr, rm)
                    os_ += [nd[0:8] * ra, nd[8:16] * ra, nd[16:24] * rm, nd[24:32] * rb, nd[32:40] * rb]
                yield
            o = jnp.concatenate(os_, axis=0).astype(bf16)
            x1 = xT[c] + _dot(woT[...], o)
            yield
            xn1 = _ln(x1)
            yield
            h = _dot(w1T[...], xn1)
            yield
            hh = h * 0.5
            h = (hh + hh * jnp.tanh(hh)).astype(bf16) if SILU_TANH else (h * jax.nn.sigmoid(h)).astype(bf16)
            yield
            x2 = x1 + _dot(w2T[...], h)
            yield x2

        def run(gens):
            live = list(gens)
            while live:
                nxt = []
                for g in live:
                    try:
                        next(g)
                        nxt.append(g)
                    except StopIteration:
                        pass
                live = nxt

        cps[2].wait()

        def g0(c):
            t0 = pl.multiple_of(c * T, T)
            x = xin[pl.ds(t0, T), :].astype(f32).T
            xT[c] = x
            yield from stage_a(c, x)

        def body0(i, carry):
            run([g0(i * NI + k) for k in range(NI)])
            return carry
        lax.fori_loop(0, NB, body0, 0)

        cps[3].wait()
        for kt in range(5):
            woT[128 * kt:128 * kt + 128, :] = wo_v[:, 128 * kt:128 * kt + 128].T
        cps[4].wait()
        for kt in range(F // 128):
            w1T[128 * kt:128 * kt + 128, :] = w1_v[:, 128 * kt:128 * kt + 128].T
        w1T[F - 64:F, :] = w1_v[:, F - 64:F].T
        cps[5].wait()
        for kt in range(F // 128):
            w2T[:, 128 * kt:128 * kt + 128] = w2_v[128 * kt:128 * kt + 128, :].T
        w2T[:, F - 64:F] = w2_v[F - 64:F, :].T
        finalize()

        def g1(c):
            x2 = yield from _last(stage_bc(c))
            xT[c] = x2
            yield from stage_a(c, x2)

        def body1(i, carry):
            run([g1(i * NI + k) for k in range(NI)])
            return carry
        lax.fori_loop(0, NB, body1, 0)
        finalize()

        def ocp(c):
            t0 = pl.multiple_of(c * T, T)
            return pltpu.make_async_copy(outv.at[pl.ds(t0, T)], o_hbm.at[pl.ds(t0, T)], osems.at[c])

        def g2(c):
            x2 = yield from _last(stage_bc(c))
            t0 = pl.multiple_of(c * T, T)
            outv[pl.ds(t0, T), :] = x2.T.astype(bf16)
            ocp(c).start()
            yield

        def body2(i, carry):
            run([g2(i * NI + k) for k in range(NI)])
            return carry
        lax.fori_loop(0, NB, body2, 0)
        for c in range(NC):
            ocp(c).wait()

    any_spec = pl.BlockSpec(memory_space=pl.ANY)
    return pl.pallas_call(
        kernel,
        out_shape=jax.ShapeDtypeStruct((S, D), bf16),
        in_specs=[any_spec] * 6,
        out_specs=any_spec,
        scratch_shapes=[
            pltpu.VMEM((S, D), bf16), pltpu.VMEM((D, 3 * D), bf16), pltpu.VMEM((H, DH, DH), bf16),
            pltpu.VMEM((D, D), bf16), pltpu.VMEM((D, F), bf16), pltpu.VMEM((F, D), bf16),
            pltpu.VMEM((D, D), bf16), pltpu.VMEM((2 * D, D), bf16), pltpu.VMEM((D, D), bf16),
            pltpu.VMEM((F, D), bf16), pltpu.VMEM((D, F), bf16),
            pltpu.VMEM((S // T, D, T), f32), pltpu.VMEM((S // T, D, T), bf16),
            pltpu.VMEM((NP, 48, 2 * PR), f32), pltpu.VMEM((NP, 48, 2 * PR), bf16),
            pltpu.VMEM((D, DH), f32), pltpu.VMEM((S, D), bf16),
            pltpu.SemaphoreType.DMA((6,)), pltpu.SemaphoreType.DMA((S // T,)),
        ],
        compiler_params=pltpu.CompilerParams(vmem_limit_bytes=110 << 20),
    )


SILU_TANH = False


def _last(g):
    last = None
    for v in g:
        last = v
        yield
    return last


_call = make()


@jax.jit
def pallas_interleave_layers__linear_kernel_hedgehog__dense_activation_silu__prompt_kernel(
    A_x: jax.Array,
    A_wqkv: jax.Array,
    A_w_phi: jax.Array,
    A_wo: jax.Array,
    B_x: jax.Array,
    B_w1: jax.Array,
    B_w2: jax.Array,
):
    o = _call(A_x.reshape(S, D), A_wqkv, A_w_phi, A_wo, B_w1, B_w2)
    return o.reshape(1, S, D)
```

```python
import jax
import jax.numpy as jnp
from jax import lax
import jax.experimental.pallas as pl
import jax.experimental.pallas.tpu as pltpu

S, D, F, H, DH = 2048, 640, 1728, 32, 20
NP = H // 2
PR = 2 * DH
KT = D // 128
LOG2E = 1.4426950408889634
f32, bf16, i32 = jnp.float32, jnp.bfloat16, jnp.int32
NN = (((1,), (0,)), ((), ()))
NT = (((1,), (1,)), ((), ()))


def _win(kt):
    lo = ((128 * kt) // PR) * PR
    hi = -((-128 * (kt + 1)) // PR) * PR
    return (lo // 16) * 16, min(-((-hi) // 16) * 16, D)


WMAX = max(_win(kt)[1] - _win(kt)[0] for kt in range(KT))


def _dot(a, b, dims=NN):
    return lax.dot_general(a, b, dims, preferred_element_type=f32)


def _rcp(x):
    r = pltpu.reciprocal(x, approx=True)
    return r * (2.0 - x * r)


def _ln(x):
    m = jnp.sum(x, axis=0, keepdims=True) * (1.0 / D)
    d = x - m
    v = jnp.sum(d * d, axis=0, keepdims=True) * (1.0 / D)
    return (d * lax.rsqrt(v + 1e-5)).astype(bf16)


def _par_reduce(v, op):
    v = op(v, pltpu.roll(v, 4, 0))
    return op(v, pltpu.roll(v, 2, 0))


def _chain(op, xs):
    r = xs[0]
    for v in xs[1:]:
        r = op(r, v)
    return r


def _phi(s):
    sl = [s[8 * i:8 * i + 8] for i in range(PR // 8)]
    mx = _par_reduce(_chain(jnp.maximum, sl), jnp.maximum)
    mn = _par_reduce(_chain(jnp.minimum, sl), jnp.minimum)
    ep = [jnp.exp2(v - mx) for v in sl]
    en = [jnp.exp2(mn - v) for v in sl]
    rp = _rcp(_par_reduce(_chain(jnp.add, ep), jnp.add))
    rn = _rcp(_par_reduce(_chain(jnp.add, en), jnp.add))
    return jnp.concatenate([v * rp for v in ep] + [v * rn for v in en], axis=0).astype(bf16)


def make(T=512, RB=320, V0=0, X1=3):
    NC = S // T

    def kernel(x_hbm, wqkv_hbm, wphi_hbm, wo_hbm, w1_hbm, w2_hbm, o_hbm,
               xin, wqkv_v, wphi_v, wo_v, w2_v, wqT, wkvT, woT, w1T, w2T,
               xT, xnT, phik, vt, kvb, scr, bdw, outv, sems, xsems, osems, psems):
        def wcp(k):
            c = slice(D * k, D * (k + 1))
            return pltpu.make_async_copy(wqkv_hbm.at[:, c], wqkv_v.at[:, c], psems.at[k])

        def xcp(c):
            t0 = pl.multiple_of(c * T, T)
            return pltpu.make_async_copy(x_hbm.at[pl.ds(t0, T)], xin.at[pl.ds(t0, T)], xsems.at[c])

        def ocp(c):
            t0 = pl.multiple_of(c * T, T)
            return pltpu.make_async_copy(outv.at[pl.ds(t0, T)], o_hbm.at[pl.ds(t0, T)], osems.at[c])

        cp_phi = pltpu.make_async_copy(wphi_hbm, wphi_v, sems.at[0])
        cp_wo = pltpu.make_async_copy(wo_hbm, wo_v, sems.at[1])
        cp_w1 = pltpu.make_async_copy(w1_hbm, w1T, sems.at[2])
        cp_w2 = pltpu.make_async_copy(w2_hbm, w2_v, sems.at[3])
        cp_phi.start()
        wcp(1).start()
        xcp(0).start()
        if V0:
            wcp(2).start()

        cp_phi.wait()
        eye = jnp.where(lax.broadcasted_iota(i32, (H, H), 0) == lax.broadcasted_iota(i32, (H, H), 1), 1.0, 0.0).astype(bf16)
        for d in range(DH):
            scr[pl.ds(d, H, stride=DH), :] = _dot(eye, wphi_v[d], NT)
        for kt in range(KT):
            lo, hi = _win(kt)
            wl = hi - lo
            r = lax.broadcasted_iota(i32, (wl, DH), 0) + lo
            p = ((r.astype(f32) + 0.5) * (1.0 / PR)).astype(i32)
            et = jnp.where(((r - p * PR) >> 1) == lax.broadcasted_iota(i32, (wl, DH), 1), 1.0, 0.0).astype(bf16)
            bd = _dot(et, scr[128 * kt:128 * kt + 128, :].astype(bf16), NT)
            r2 = lax.broadcasted_iota(i32, (wl, 128), 0) + lo
            c2 = lax.broadcasted_iota(i32, (wl, 128), 1) + 128 * kt
            p2 = ((r2.astype(f32) + 0.5) * (1.0 / PR)).astype(i32)
            h2 = ((c2.astype(f32) + 0.5) * (1.0 / DH)).astype(i32)
            bdw[kt, 0:wl, :] = jnp.where((p2 * 2 + (r2 & 1)) == h2, bd, 0.0).astype(bf16)

        def fold(k, dst, j):
            parts = [_dot(bdw[kt, 0:_win(kt)[1] - _win(kt)[0], :],
                          wqkv_v[128 * j:128 * (j + 1), D * k + 128 * kt:D * k + 128 * (kt + 1)], NT)
                     for kt in range(KT)]
            for b in range(0, D, 16):
                acc = _chain(jnp.add, [parts[kt][b - _win(kt)[0]:b - _win(kt)[0] + 16]
                                       for kt in range(KT) if _win(kt)[0] <= b < _win(kt)[1]])
                dst[b:b + 16, 128 * j:128 * (j + 1)] = (acc * LOG2E).astype(bf16)

        def load_x(c):
            x = xin[pl.ds(pl.multiple_of(c * T, T), T), :].astype(f32).T
            xT[c] = x
            xnT[c] = _ln(x)

        ones8 = jnp.ones((8, T), f32)

        def stage_a(c):
            xn = xnT[c]
            for r0 in range(0, D, RB):
                pk = _dot(wkvT[r0:r0 + RB, :], xn)
                for j in range(RB // PR):
                    p = r0 // PR + j
                    phik[c, 2 * PR * p:2 * PR * (p + 1), :] = _phi(pk[PR * j:PR * j + PR])
            for r0 in range(0, D, RB):
                vv = _dot(wkvT[D + r0:D + r0 + RB, :], xn)
                for j in range(RB // PR):
                    p = r0 // PR + j
                    vt[c, 48 * p:48 * (p + 1), :] = jnp.concatenate([vv[PR * j:PR * j + PR], ones8], axis=0).astype(bf16)

        def finalize():
            r = lax.broadcasted_iota(i32, (48, 2 * PR), 0)
            cc = lax.broadcasted_iota(i32, (48, 2 * PR), 1)
            hsel = jnp.where(r < PR, jnp.where(r >= DH, 1, 0), jnp.where(r >= PR + 4, 1, 0))
            ok = hsel == (cc & 1)
            for p in range(NP):
                m = _chain(jnp.add, [_dot(vt[c, 48 * p:48 * (p + 1), :], phik[c, 2 * PR * p:2 * PR * (p + 1), :], NT)
                                     for c in range(NC)])
                kvb[p] = jnp.where(ok, m, 0.0).astype(bf16)

        low4 = lax.broadcasted_iota(i32, (8, T), 0) < 4

        def stage_bc(c):
            xn = xnT[c]
            os_ = []
            for r0 in range(0, D, RB):
                pq = _dot(wqT[r0:r0 + RB, :], xn)
                for j in range(RB // PR):
                    nd = _dot(kvb[r0 // PR + j], _phi(pq[PR * j:PR * j + PR]))
                    rm = _rcp(nd[PR:PR + 8] + 1e-6)
                    rr = pltpu.roll(rm, 4, 0)
                    ra = jnp.where(low4, rm, rr)
                    rb = jnp.where(low4, rr, rm)
                    os_ += [nd[0:8] * ra, nd[8:16] * ra, nd[16:24] * rm, nd[24:32] * rb, nd[32:40] * rb]
            o = jnp.concatenate(os_, axis=0).astype(bf16)
            x1 = xT[c] + _dot(woT[...], o)
            h = _dot(w1T[...], _ln(x1))
            hh = h * 0.5
            h = (hh + hh * jnp.tanh(hh)).astype(bf16)
            x2 = x1 + _dot(w2T[...], h)
            xT[c] = x2
            xnT[c] = _ln(x2)
            outv[pl.ds(pl.multiple_of(c * T, T), T), :] = x2.T.astype(bf16)

        if not V0:
            wcp(2).start()
        xcp(0).wait()
        wcp(1).wait()
        for c in range(1, X1):
            xcp(c).start()
        for j in range(KT):
            fold(1, wkvT, j)
        load_x(0)
        wcp(2).wait()
        for c in range(X1, NC):
            xcp(c).start()
        wcp(0).start()
        cp_wo.start()
        cp_w1.start()
        cp_w2.start()
        for j in range(KT):
            wkvT[D + 128 * j:D + 128 * (j + 1), :] = wqkv_v[:, 2 * D + 128 * j:2 * D + 128 * (j + 1)].T

        def body_a0(i, carry):
            @pl.when(i < NC - 1)
            def _():
                xcp(i + 1).wait()
            stage_a(i)
            load_x(jnp.minimum(i + 1, NC - 1))
            return carry
        lax.fori_loop(0, NC, body_a0, 0)

        wcp(0).wait()
        cp_wo.wait()
        cp_w1.wait()
        cp_w2.wait()
        for j in range(KT):
            fold(0, wqT, j)
        for j in range(KT):
            woT[128 * j:128 * (j + 1), :] = wo_v[:, 128 * j:128 * (j + 1)].T
        for j in range(F // 128):
            w2T[:, 128 * j:128 * (j + 1)] = w2_v[128 * j:128 * (j + 1), :].T
        w2T[:, F - F % 128:F] = w2_v[F - F % 128:F, :].T
        finalize()

        def layer(l, carry):
            def body_bc(i, carry):
                stage_bc(i)

                @pl.when(l == 1)
                def _():
                    ocp(i).start()
                return carry
            lax.fori_loop(0, NC, body_bc, 0)

            @pl.when(l == 0)
            def _():
                def body_a(i, carry):
                    stage_a(i)
                    return carry
                lax.fori_loop(0, NC, body_a, 0)
                finalize()
            return carry
        lax.fori_loop(0, 2, layer, 0)
        for c in range(NC):
            ocp(c).wait()

    hbm = pl.BlockSpec(memory_space=pltpu.HBM)
    return pl.pallas_call(
        kernel,
        out_shape=jax.ShapeDtypeStruct((S, D), bf16),
        in_specs=[hbm] * 6,
        out_specs=hbm,
        scratch_shapes=[
            pltpu.VMEM((S, D), bf16), pltpu.VMEM((D, 3 * D), bf16), pltpu.VMEM((DH, DH, H), bf16),
            pltpu.VMEM((D, D), bf16), pltpu.VMEM((F, D), bf16),
            pltpu.VMEM((D, D), bf16), pltpu.VMEM((2 * D, D), bf16), pltpu.VMEM((D, D), bf16),
            pltpu.VMEM((F, D), bf16), pltpu.VMEM((D, F), bf16),
            pltpu.VMEM((NC, D, T), f32), pltpu.VMEM((NC, D, T), bf16),
            pltpu.VMEM((NC, NP * 2 * PR, T), bf16), pltpu.VMEM((NC, NP * 48, T), bf16),
            pltpu.VMEM((NP, 48, 2 * PR), bf16),
            pltpu.VMEM((D, DH), f32), pltpu.VMEM((KT, WMAX, 128), bf16), pltpu.VMEM((S, D), bf16),
            pltpu.SemaphoreType.DMA((4,)), pltpu.SemaphoreType.DMA((NC,)), pltpu.SemaphoreType.DMA((NC,)),
            pltpu.SemaphoreType.DMA((3,)),
        ],
        compiler_params=pltpu.CompilerParams(vmem_limit_bytes=100 << 20),
    )


_call = make(X1=2)


@jax.jit
def pallas_interleave_layers__linear_kernel_hedgehog__dense_activation_silu__prompt_kernel(
    A_x: jax.Array,
    A_wqkv: jax.Array,
    A_w_phi: jax.Array,
    A_wo: jax.Array,
    B_x: jax.Array,
    B_w1: jax.Array,
    B_w2: jax.Array,
):
    o = _call(A_x.reshape(S, D), A_wqkv, A_w_phi.transpose(1, 2, 0), A_wo, B_w1.T, B_w2)
    return o.reshape(1, S, D)
```

```python
import jax
import jax.numpy as jnp
from jax import lax
import jax.experimental.pallas as pl
import jax.experimental.pallas.tpu as pltpu

S, D, F, H, DH = 2048, 640, 1728, 32, 20
NP = H // 2
PR = 2 * DH
PB = 48
KT = D // 128
T = 512
NC = S // T
LOG2E = 1.4426950408889634
f32, bf16, i32 = jnp.float32, jnp.bfloat16, jnp.int32
NN = (((1,), (0,)), ((), ()))
NT = (((1,), (1,)), ((), ()))


def _win(kt):
    lo = ((128 * kt) // PR) * PR
    hi = -((-128 * (kt + 1)) // PR) * PR
    return (lo // 16) * 16, min(-((-hi) // 16) * 16, D)


WMAX = max(_win(kt)[1] - _win(kt)[0] for kt in range(KT))


def _dot(a, b, dims=NN):
    return lax.dot_general(a, b, dims, preferred_element_type=f32)


def _rcp(x):
    r = pltpu.reciprocal(x, approx=True)
    return r * (2.0 - x * r)


def _ln(x):
    m = jnp.sum(x, axis=0, keepdims=True) * (1.0 / D)
    d = x - m
    v = jnp.sum(d * d, axis=0, keepdims=True) * (1.0 / D)
    return (d * lax.rsqrt(v + 1e-5)).astype(bf16)


def _stats(x):
    m = jnp.sum(x, axis=0, keepdims=True) * (1.0 / D)
    v = jnp.maximum(jnp.sum(x * x, axis=0, keepdims=True) * (1.0 / D) - m * m, 0.0)
    r = lax.rsqrt(v + 1e-5)
    return r, r * m


def _par_reduce(v, op):
    v = op(v, pltpu.roll(v, 4, 0))
    return op(v, pltpu.roll(v, 2, 0))


def _chain(op, xs):
    r = xs[0]
    for v in xs[1:]:
        r = op(r, v)
    return r


def _phi(s):
    sl = [s[8 * i:8 * i + 8] for i in range(PR // 8)]
    mx = _par_reduce(_chain(jnp.maximum, sl), jnp.maximum)
    mn = _par_reduce(_chain(jnp.minimum, sl), jnp.minimum)
    ep = [jnp.exp2(v - mx) for v in sl]
    en = [jnp.exp2(mn - v) for v in sl]
    rp = _rcp(_par_reduce(_chain(jnp.add, ep), jnp.add))
    rn = _rcp(_par_reduce(_chain(jnp.add, en), jnp.add))
    return jnp.concatenate([v * rp for v in ep] + [v * rn for v in en], axis=0).astype(bf16)


def _kernel(x_hbm, wqkv_hbm, wphi_hbm, wo_hbm, w1_hbm, w2_hbm, o_hbm,
            xin, wqkv_v, wphi_v, wo_v, w2_v, wqT, wkvT, woT, w1T, w2T,
            xT, phik, vt, kvb, rs, aux, csv, scr, bdw, outv, sems, wsems, xsems, osems):
    def wcp(k):
        c = slice(D * k, D * (k + 1))
        return pltpu.make_async_copy(wqkv_hbm.at[:, c], wqkv_v.at[:, c], wsems.at[k])

    def xcp(c):
        t0 = pl.multiple_of(c * T, T)
        return pltpu.make_async_copy(x_hbm.at[pl.ds(t0, T)], xin.at[pl.ds(t0, T)], xsems.at[c])

    def ocp(c):
        t0 = pl.multiple_of(c * T, T)
        return pltpu.make_async_copy(outv.at[pl.ds(t0, T)], o_hbm.at[pl.ds(t0, T)], osems.at[c])

    cp_phi = pltpu.make_async_copy(wphi_hbm, wphi_v, sems.at[0])
    cp_wo = pltpu.make_async_copy(wo_hbm, wo_v, sems.at[1])
    cp_w1 = pltpu.make_async_copy(w1_hbm, w1T, sems.at[2])
    cp_w2 = pltpu.make_async_copy(w2_hbm, w2_v, sems.at[3])

    cp_phi.start()
    wcp(1).start()
    cp_phi.wait()
    xcp(0).start()
    wcp(2).start()

    eye = jnp.where(lax.broadcasted_iota(i32, (H, H), 0) == lax.broadcasted_iota(i32, (H, H), 1),
                    1.0, 0.0).astype(bf16)
    for d in range(DH):
        scr[pl.ds(d, H, stride=DH), :] = _dot(eye, wphi_v[d], NT)
    for kt in range(KT):
        lo, hi = _win(kt)
        wl = hi - lo
        r = lax.broadcasted_iota(i32, (wl, DH), 0) + lo
        p = ((r.astype(f32) + 0.5) * (1.0 / PR)).astype(i32)
        et = jnp.where(((r - p * PR) >> 1) == lax.broadcasted_iota(i32, (wl, DH), 1), 1.0, 0.0).astype(bf16)
        bd = _dot(et, scr[128 * kt:128 * kt + 128, :].astype(bf16), NT)
        r2 = lax.broadcasted_iota(i32, (wl, 128), 0) + lo
        c2 = lax.broadcasted_iota(i32, (wl, 128), 1) + 128 * kt
        p2 = ((r2.astype(f32) + 0.5) * (1.0 / PR)).astype(i32)
        h2 = ((c2.astype(f32) + 0.5) * (1.0 / DH)).astype(i32)
        bdw[kt, 0:wl, :] = jnp.where((p2 * 2 + (r2 & 1)) == h2, bd, 0.0).astype(bf16)

    def fold(k, dst):
        parts = [_dot(bdw[kt, 0:_win(kt)[1] - _win(kt)[0], :],
                      wqkv_v[:, D * k + 128 * kt:D * k + 128 * (kt + 1)], NT) for kt in range(KT)]
        for b in range(0, D, 16):
            acc = _chain(jnp.add, [parts[kt][b - _win(kt)[0]:b - _win(kt)[0] + 16]
                                   for kt in range(KT) if _win(kt)[0] <= b < _win(kt)[1]])
            acc = acc - jnp.sum(acc, axis=1, keepdims=True) * (1.0 / D)
            dst[b:b + 16, :] = (acc * LOG2E).astype(bf16)

    row8 = lax.broadcasted_iota(i32, (8, T), 0)

    def put_stats(c, x):
        r, rm = _stats(x)
        rs[c] = jnp.broadcast_to(r, (8, T))
        aux[c] = jnp.where(row8 == 0, 1.0, rm)

    def load_x(c):
        x = xin[pl.ds(pl.multiple_of(c * T, T), T), :].T
        xT[c] = x
        put_stats(c, x.astype(f32))

    def rstd_rows(c):
        return jnp.concatenate([rs[c]] * (D // 8), axis=0)

    def stage_a(c):
        x = xT[c]
        r = rstd_rows(c)
        a8 = aux[c]
        pk = _dot(wkvT[0:D, :], x) * r
        for p in range(NP):
            phik[c, 2 * PR * p:2 * PR * (p + 1), :] = _phi(pk[PR * p:PR * (p + 1)])
        vv = _dot(wkvT[D:2 * D, :], x) * r
        for p in range(NP):
            vt[c, PB * p:PB * (p + 1), :] = jnp.concatenate([vv[PR * p:PR * (p + 1)], a8], axis=0).astype(bf16)

    def finalize():
        r = lax.broadcasted_iota(i32, (PB, 2 * PR), 0)
        cc = lax.broadcasted_iota(i32, (PB, 2 * PR), 1)
        hsel = jnp.where(r < PR, jnp.where(r >= DH, 1, 0), jnp.where(r >= PR + 4, 1, 0))
        ok = hsel == (cc & 1)
        for p in range(NP):
            m = _chain(jnp.add, [_dot(vt[c, PB * p:PB * (p + 1), :], phik[c, 2 * PR * p:2 * PR * (p + 1), :], NT)
                                 for c in range(NC)])
            kv = m[0:PR] - csv[PR * p:PR * (p + 1), 0:2 * PR] * m[PR + 1:PR + 2]
            zz = jnp.broadcast_to(m[PR:PR + 1], (8, 2 * PR))
            kvb[p] = jnp.where(ok, jnp.concatenate([kv, zz], axis=0), 0.0).astype(bf16)

    low4 = row8 < 4

    def stage_bc(c):
        x = xT[c]
        pq = _dot(wqT[...], x) * rstd_rows(c)
        os_ = []
        for p in range(NP):
            nd = _dot(kvb[p], _phi(pq[PR * p:PR * (p + 1)]))
            rm = _rcp(nd[PR:PB] + 1e-6)
            rr = pltpu.roll(rm, 4, 0)
            ra = jnp.where(low4, rm, rr)
            rb = jnp.where(low4, rr, rm)
            os_ += [nd[0:8] * ra, nd[8:16] * ra, nd[16:24] * rm, nd[24:32] * rb, nd[32:40] * rb]
        o = jnp.concatenate(os_, axis=0).astype(bf16)
        x1 = x.astype(f32) + _dot(woT[...], o)
        hh = _dot(w1T[...], _ln(x1)) * 0.5
        h = (hh + hh * jnp.tanh(hh)).astype(bf16)
        x2 = x1 + _dot(w2T[...], h)
        xb = x2.astype(bf16)
        xT[c] = xb
        put_stats(c, x2)
        outv[pl.ds(pl.multiple_of(c * T, T), T), :] = xb.T

    wcp(1).wait()
    fold(1, wkvT)
    xcp(0).wait()
    xcp(1).start()
    load_x(0)
    wcp(2).wait()
    for c in range(2, NC):
        xcp(c).start()
    wcp(0).start()
    cp_wo.start()
    cp_w1.start()
    cp_w2.start()
    for j in range(KT):
        wkvT[D + 128 * j:D + 128 * (j + 1), :] = wqkv_v[:, 2 * D + 128 * j:2 * D + 128 * (j + 1)].T

    def body_a0(i, carry):
        @pl.when(i < NC - 1)
        def _():
            xcp(i + 1).wait()
        stage_a(i)
        load_x(jnp.minimum(i + 1, NC - 1))
        return carry
    lax.fori_loop(0, NC, body_a0, 0)

    wcp(0).wait()
    cp_wo.wait()
    cp_w1.wait()
    cp_w2.wait()
    fold(0, wqT)
    csv[...] = jnp.broadcast_to(jnp.sum(wkvT[D:2 * D, :].astype(f32), axis=1, keepdims=True), (D, 128))
    for j in range(KT):
        woT[128 * j:128 * (j + 1), :] = wo_v[:, 128 * j:128 * (j + 1)].T
    for j in range(F // 128):
        w2T[:, 128 * j:128 * (j + 1)] = w2_v[128 * j:128 * (j + 1), :].T
    w2T[:, F - F % 128:F] = w2_v[F - F % 128:F, :].T
    finalize()

    def layer(l, carry):
        def body_bc(i, carry):
            stage_bc(i)

            @pl.when(l == 1)
            def _():
                ocp(i).start()
            return carry
        lax.fori_loop(0, NC, body_bc, 0)

        @pl.when(l == 0)
        def _():
            def body_a(i, carry):
                stage_a(i)
                return carry
            lax.fori_loop(0, NC, body_a, 0)
            finalize()
        return carry
    lax.fori_loop(0, 2, layer, 0)
    for c in range(NC):
        ocp(c).wait()


def _make_call():
    hbm = pl.BlockSpec(memory_space=pltpu.HBM)
    return pl.pallas_call(
        _kernel,
        out_shape=jax.ShapeDtypeStruct((S, D), bf16),
        in_specs=[hbm] * 6,
        out_specs=hbm,
        scratch_shapes=[
            pltpu.VMEM((S, D), bf16),
            pltpu.VMEM((D, 3 * D), bf16),
            pltpu.VMEM((DH, DH, H), bf16),
            pltpu.VMEM((D, D), bf16),
            pltpu.VMEM((F, D), bf16),
            pltpu.VMEM((D, D), bf16),
            pltpu.VMEM((2 * D, D), bf16),
            pltpu.VMEM((D, D), bf16),
            pltpu.VMEM((F, D), bf16),
            pltpu.VMEM((D, F), bf16),
            pltpu.VMEM((NC, D, T), bf16),
            pltpu.VMEM((NC, NP * 2 * PR, T), bf16),
            pltpu.VMEM((NC, NP * PB, T), bf16),
            pltpu.VMEM((NP, PB, 2 * PR), bf16),
            pltpu.VMEM((NC, 8, T), f32),
            pltpu.VMEM((NC, 8, T), f32),
            pltpu.VMEM((D, 128), f32),
            pltpu.VMEM((D, DH), f32),
            pltpu.VMEM((KT, WMAX, 128), bf16),
            pltpu.VMEM((S, D), bf16),
            pltpu.SemaphoreType.DMA((4,)),
            pltpu.SemaphoreType.DMA((3,)),
            pltpu.SemaphoreType.DMA((NC,)),
            pltpu.SemaphoreType.DMA((NC,)),
        ],
        compiler_params=pltpu.CompilerParams(vmem_limit_bytes=100 << 20),
    )


@jax.jit
def pallas_interleave_layers__linear_kernel_hedgehog__dense_activation_silu__prompt_kernel(
    A_x: jax.Array,
    A_wqkv: jax.Array,
    A_w_phi: jax.Array,
    A_wo: jax.Array,
    B_x: jax.Array,
    B_w1: jax.Array,
    B_w2: jax.Array,
):
    o = _make_call()(A_x.reshape(S, D), A_wqkv, A_w_phi.transpose(1, 2, 0), A_wo, B_w1.T, B_w2)
    return o.reshape(1, S, D)
```

```python
import jax
import jax.numpy as jnp
from jax import lax
import jax.experimental.pallas as pl
import jax.experimental.pallas.tpu as pltpu

S, D, F, H, DH = 2048, 640, 1728, 32, 20
NP = H // 2
PR = 2 * DH
PB = 48
KT = D // 128
T = 512
NC = S // T
LOG2E = 1.4426950408889634
f32, bf16, i32 = jnp.float32, jnp.bfloat16, jnp.int32
NN = (((1,), (0,)), ((), ()))
NT = (((1,), (1,)), ((), ()))


def _win(kt):
    lo = ((128 * kt) // PR) * PR
    hi = -((-128 * (kt + 1)) // PR) * PR
    return (lo // 16) * 16, min(-((-hi) // 16) * 16, D)


WMAX = max(_win(kt)[1] - _win(kt)[0] for kt in range(KT))


def _dot(a, b, dims=NN):
    return lax.dot_general(a, b, dims, preferred_element_type=f32)


def _rcp(x):
    r = pltpu.reciprocal(x, approx=True)
    return r * (2.0 - x * r)


def _ln(x, scale):
    m = jnp.sum(x, axis=0, keepdims=True) * (1.0 / D)
    d = x - m
    v = jnp.sum(d * d, axis=0, keepdims=True) * (1.0 / D)
    return (d * (scale * lax.rsqrt(v + 1e-5))).astype(bf16)


def _stats(x):
    m = jnp.sum(x, axis=0, keepdims=True) * (1.0 / D)
    v = jnp.maximum(jnp.sum(x * x, axis=0, keepdims=True) * (1.0 / D) - m * m, 0.0)
    r = lax.rsqrt(v + 1e-5)
    return r, r * m


def _par_reduce(v, op):
    v = op(v, pltpu.roll(v, 4, 0))
    return op(v, pltpu.roll(v, 2, 0))


def _chain(op, xs):
    r = xs[0]
    for v in xs[1:]:
        r = op(r, v)
    return r


def _phi(s):
    sl = [s[8 * i:8 * i + 8] for i in range(PR // 8)]
    mx = _par_reduce(_chain(jnp.maximum, sl), jnp.maximum)
    mn = _par_reduce(_chain(jnp.minimum, sl), jnp.minimum)
    ep = [jnp.exp2(v - mx) for v in sl]
    en = [jnp.exp2(mn - v) for v in sl]
    rp = _rcp(_par_reduce(_chain(jnp.add, ep), jnp.add))
    rn = _rcp(_par_reduce(_chain(jnp.add, en), jnp.add))
    return jnp.concatenate([v * rp for v in ep] + [v * rn for v in en], axis=0).astype(bf16)


def _kernel(x_hbm, wqkv_hbm, wphi_hbm, wo_hbm, w1_hbm, w2_hbm, o_hbm,
            xin, wqkv_v, wphi_v, wo_v, w2_v, wqT, wkvT, woT, w1T, w2T,
            xT, phik, vt, kvb, rs, aux, csv, scr, bdw, outv, sems, wsems, xsems, osems):
    def wcp(k):
        c = slice(D * k, D * (k + 1))
        return pltpu.make_async_copy(wqkv_hbm.at[:, c], wqkv_v.at[:, c], wsems.at[k])

    def xcp(c):
        t0 = pl.multiple_of(c * T, T)
        return pltpu.make_async_copy(x_hbm.at[pl.ds(t0, T)], xin.at[pl.ds(t0, T)], xsems.at[c])

    def ocp(c):
        t0 = pl.multiple_of(c * T, T)
        return pltpu.make_async_copy(outv.at[pl.ds(t0, T)], o_hbm.at[pl.ds(t0, T)], osems.at[c])

    cp_phi = pltpu.make_async_copy(wphi_hbm, wphi_v, sems.at[0])
    cp_wo = pltpu.make_async_copy(wo_hbm, wo_v, sems.at[1])
    cp_w1 = pltpu.make_async_copy(w1_hbm, w1T, sems.at[2])
    cp_w2 = pltpu.make_async_copy(w2_hbm, w2_v, sems.at[3])

    cp_phi.start()
    wcp(1).start()
    cp_phi.wait()
    xcp(0).start()

    eye = jnp.where(lax.broadcasted_iota(i32, (H, H), 0) == lax.broadcasted_iota(i32, (H, H), 1),
                    1.0, 0.0).astype(bf16)
    for d in range(DH):
        scr[pl.ds(d, H, stride=DH), :] = _dot(eye, wphi_v[d], NT)
    for kt in range(KT):
        lo, hi = _win(kt)
        wl = hi - lo
        r = lax.broadcasted_iota(i32, (wl, DH), 0) + lo
        p = ((r.astype(f32) + 0.5) * (1.0 / PR)).astype(i32)
        et = jnp.where(((r - p * PR) >> 1) == lax.broadcasted_iota(i32, (wl, DH), 1), 1.0, 0.0).astype(bf16)
        bd = _dot(et, scr[128 * kt:128 * kt + 128, :].astype(bf16), NT)
        r2 = lax.broadcasted_iota(i32, (wl, 128), 0) + lo
        c2 = lax.broadcasted_iota(i32, (wl, 128), 1) + 128 * kt
        p2 = ((r2.astype(f32) + 0.5) * (1.0 / PR)).astype(i32)
        h2 = ((c2.astype(f32) + 0.5) * (1.0 / DH)).astype(i32)
        bdw[kt, 0:wl, :] = jnp.where((p2 * 2 + (r2 & 1)) == h2, bd, 0.0).astype(bf16)

    def fold(k, dst):
        parts = [_dot(bdw[kt, 0:_win(kt)[1] - _win(kt)[0], :],
                      wqkv_v[:, D * k + 128 * kt:D * k + 128 * (kt + 1)], NT) for kt in range(KT)]
        for b in range(0, D, 16):
            acc = _chain(jnp.add, [parts[kt][b - _win(kt)[0]:b - _win(kt)[0] + 16]
                                   for kt in range(KT) if _win(kt)[0] <= b < _win(kt)[1]])
            acc = acc - jnp.sum(acc, axis=1, keepdims=True) * (1.0 / D)
            dst[b:b + 16, :] = (acc * LOG2E).astype(bf16)

    row8 = lax.broadcasted_iota(i32, (8, T), 0)

    def put_stats(c, x):
        r, rm = _stats(x)
        rs[c] = jnp.broadcast_to(r, (8, T))
        aux[c] = jnp.where(row8 == 0, 1.0, rm)

    def load_x(c):
        x = xin[pl.ds(pl.multiple_of(c * T, T), T), :].T
        xT[c] = x
        put_stats(c, x.astype(f32))

    def rstd_rows(c):
        return jnp.concatenate([rs[c]] * (D // 8), axis=0)

    def stage_k(c, x, r):
        pk = _dot(wkvT[0:D, :], x) * r
        for p in range(NP):
            phik[c, 2 * PR * p:2 * PR * (p + 1), :] = _phi(pk[PR * p:PR * (p + 1)])

    def stage_v(c, x, r):
        a8 = aux[c]
        vv = _dot(wkvT[D:2 * D, :], x) * r
        for p in range(NP):
            vt[c, PB * p:PB * (p + 1), :] = jnp.concatenate([vv[PR * p:PR * (p + 1)], a8], axis=0).astype(bf16)

    def stage_a(c):
        x = xT[c]
        r = rstd_rows(c)
        stage_k(c, x, r)
        stage_v(c, x, r)

    def finalize():
        r = lax.broadcasted_iota(i32, (PB, 2 * PR), 0)
        cc = lax.broadcasted_iota(i32, (PB, 2 * PR), 1)
        hsel = jnp.where(r < PR, jnp.where(r >= DH, 1, 0), jnp.where(r >= PR + 4, 1, 0))
        ok = hsel == (cc & 1)
        for p in range(NP):
            m = _chain(jnp.add, [_dot(vt[c, PB * p:PB * (p + 1), :], phik[c, 2 * PR * p:2 * PR * (p + 1), :], NT)
                                 for c in range(NC)])
            kv = m[0:PR] - csv[PR * p:PR * (p + 1), 0:2 * PR] * m[PR + 1:PR + 2]
            zz = jnp.broadcast_to(m[PR:PR + 1], (8, 2 * PR))
            kvb[p] = jnp.where(ok, jnp.concatenate([kv, zz], axis=0), 0.0).astype(bf16)

    low4 = row8 < 4

    def stage_bc(c):
        x = xT[c]
        pq = _dot(wqT[...], x) * rstd_rows(c)
        os_ = []
        for p in range(NP):
            nd = _dot(kvb[p], _phi(pq[PR * p:PR * (p + 1)]))
            rm = _rcp(nd[PR:PB] + 1e-6)
            rr = pltpu.roll(rm, 4, 0)
            ra = jnp.where(low4, rm, rr)
            rb = jnp.where(low4, rr, rm)
            os_ += [nd[0:8] * ra, nd[8:16] * ra, nd[16:24] * rm, nd[24:32] * rb, nd[32:40] * rb]
        o = jnp.concatenate(os_, axis=0).astype(bf16)
        x1 = x.astype(f32) + _dot(woT[...], o)
        hh = _dot(w1T[...], _ln(x1, 0.5))
        h = (hh + hh * jnp.tanh(hh)).astype(bf16)
        x2 = x1 + _dot(w2T[...], h)
        xb = x2.astype(bf16)
        xT[c] = xb
        put_stats(c, x2)
        outv[pl.ds(pl.multiple_of(c * T, T), T), :] = x2.T.astype(bf16)

    wcp(1).wait()
    wcp(2).start()
    fold(1, wkvT)
    xcp(0).wait()
    xcp(1).start()
    wcp(0).start()
    load_x(0)
    stage_k(0, xT[0], rstd_rows(0))
    wcp(2).wait()
    wcp(0).wait()
    xcp(1).wait()
    for c in range(2, NC):
        xcp(c).start()
    cp_wo.start()
    cp_w1.start()
    cp_w2.start()
    for j in range(KT):
        wkvT[D + 128 * j:D + 128 * (j + 1), :] = wqkv_v[:, 2 * D + 128 * j:2 * D + 128 * (j + 1)].T
    fold(0, wqT)
    stage_v(0, xT[0], rstd_rows(0))
    load_x(1)

    def body_a0(i, carry):
        @pl.when(i < NC - 1)
        def _():
            xcp(i + 1).wait()
        stage_a(i)
        load_x(jnp.minimum(i + 1, NC - 1))
        return carry
    lax.fori_loop(1, NC, body_a0, 0)

    cp_wo.wait()
    cp_w1.wait()
    cp_w2.wait()
    csv[...] = jnp.broadcast_to(jnp.sum(wkvT[D:2 * D, :].astype(f32), axis=1, keepdims=True), (D, 128))
    for j in range(KT):
        woT[128 * j:128 * (j + 1), :] = wo_v[:, 128 * j:128 * (j + 1)].T
    for j in range(F // 128):
        w2T[:, 128 * j:128 * (j + 1)] = w2_v[128 * j:128 * (j + 1), :].T
    w2T[:, F - F % 128:F] = w2_v[F - F % 128:F, :].T
    finalize()

    def layer(l, carry):
        def body_bc(i, carry):
            stage_bc(i)

            @pl.when(l == 1)
            def _():
                ocp(i).start()
            return carry
        lax.fori_loop(0, NC, body_bc, 0)

        @pl.when(l == 0)
        def _():
            def body_a(i, carry):
                stage_a(i)
                return carry
            lax.fori_loop(0, NC, body_a, 0)
            finalize()
        return carry
    lax.fori_loop(0, 2, layer, 0)
    for c in range(NC):
        ocp(c).wait()


def _make_call():
    hbm = pl.BlockSpec(memory_space=pltpu.HBM)
    return pl.pallas_call(
        _kernel,
        out_shape=jax.ShapeDtypeStruct((S, D), bf16),
        in_specs=[hbm] * 6,
        out_specs=hbm,
        scratch_shapes=[
            pltpu.VMEM((S, D), bf16),
            pltpu.VMEM((D, 3 * D), bf16),
            pltpu.VMEM((DH, DH, H), bf16),
            pltpu.VMEM((D, D), bf16),
            pltpu.VMEM((F, D), bf16),
            pltpu.VMEM((D, D), bf16),
            pltpu.VMEM((2 * D, D), bf16),
            pltpu.VMEM((D, D), bf16),
            pltpu.VMEM((F, D), bf16),
            pltpu.VMEM((D, F), bf16),
            pltpu.VMEM((NC, D, T), bf16),
            pltpu.VMEM((NC, NP * 2 * PR, T), bf16),
            pltpu.VMEM((NC, NP * PB, T), bf16),
            pltpu.VMEM((NP, PB, 2 * PR), bf16),
            pltpu.VMEM((NC, 8, T), f32),
            pltpu.VMEM((NC, 8, T), f32),
            pltpu.VMEM((D, 128), f32),
            pltpu.VMEM((D, DH), f32),
            pltpu.VMEM((KT, WMAX, 128), bf16),
            pltpu.VMEM((S, D), bf16),
            pltpu.SemaphoreType.DMA((4,)),
            pltpu.SemaphoreType.DMA((3,)),
            pltpu.SemaphoreType.DMA((NC,)),
            pltpu.SemaphoreType.DMA((NC,)),
        ],
        compiler_params=pltpu.CompilerParams(vmem_limit_bytes=100 << 20),
    )


@jax.jit
def pallas_interleave_layers__linear_kernel_hedgehog__dense_activation_silu__prompt_kernel(
    A_x: jax.Array,
    A_wqkv: jax.Array,
    A_w_phi: jax.Array,
    A_wo: jax.Array,
    B_x: jax.Array,
    B_w1: jax.Array,
    B_w2: jax.Array,
):
    o = _make_call()(A_x.reshape(S, D), A_wqkv, A_w_phi.transpose(1, 2, 0), A_wo, B_w1.T, B_w2)
    return o.reshape(1, S, D)
```

```python
import jax
import jax.numpy as jnp
from jax import lax
import jax.experimental.pallas as pl
import jax.experimental.pallas.tpu as pltpu

S, D, F, H, DH = 2048, 640, 1728, 32, 20
NP = H // 2
PR = 2 * DH
PB = 48
KT = D // 128
T = 512
NC = S // T
LOG2E = 1.4426950408889634
f32, bf16, i32 = jnp.float32, jnp.bfloat16, jnp.int32
NN = (((1,), (0,)), ((), ()))
NT = (((1,), (1,)), ((), ()))


def _win(kt):
    lo = ((128 * kt) // PR) * PR
    hi = -((-128 * (kt + 1)) // PR) * PR
    return (lo // 16) * 16, min(-((-hi) // 16) * 16, D)


WMAX = max(_win(kt)[1] - _win(kt)[0] for kt in range(KT))


def _dot(a, b, dims=NN):
    return lax.dot_general(a, b, dims, preferred_element_type=f32)


def _rcp(x):
    r = pltpu.reciprocal(x, approx=True)
    return r * (2.0 - x * r)


def _ln(x, scale):
    m = jnp.sum(x, axis=0, keepdims=True) * (1.0 / D)
    d = x - m
    v = jnp.sum(d * d, axis=0, keepdims=True) * (1.0 / D)
    return (d * (scale * lax.rsqrt(v + 1e-5))).astype(bf16)


def _stats(x):
    d = x - jnp.sum(x[0:8], axis=0, keepdims=True) * 0.125
    m = jnp.sum(d, axis=0, keepdims=True) * (1.0 / D)
    v = jnp.maximum(jnp.sum(d * d, axis=0, keepdims=True) * (1.0 / D) - m * m, 0.0)
    r = lax.rsqrt(v + 1e-5)
    return d.astype(bf16), r, r * m


def _par_reduce(v, op):
    v = op(v, pltpu.roll(v, 4, 0))
    return op(v, pltpu.roll(v, 2, 0))


def _chain(op, xs):
    r = xs[0]
    for v in xs[1:]:
        r = op(r, v)
    return r


def _phi(s):
    sl = [s[8 * i:8 * i + 8] for i in range(PR // 8)]
    mx = _par_reduce(_chain(jnp.maximum, sl), jnp.maximum)
    mn = _par_reduce(_chain(jnp.minimum, sl), jnp.minimum)
    ep = [jnp.exp2(v - mx) for v in sl]
    en = [jnp.exp2(mn - v) for v in sl]
    rp = _rcp(_par_reduce(_chain(jnp.add, ep), jnp.add))
    rn = _rcp(_par_reduce(_chain(jnp.add, en), jnp.add))
    return jnp.concatenate([v * rp for v in ep] + [v * rn for v in en], axis=0).astype(bf16)


def _kernel(x_hbm, wqkv_hbm, wphi_hbm, wo_hbm, w1_hbm, w2_hbm, o_hbm,
            xin, wqkv_v, wphi_v, wo_v, w2_v, wqT, wkvT, woT, w1T, w2T,
            xT, dT, phik, vt, kvb, rs, aux, csv, scr, bdw, outv, sems, wsems, xsems, osems):
    def wcp(k):
        c = slice(D * k, D * (k + 1))
        return pltpu.make_async_copy(wqkv_hbm.at[:, c], wqkv_v.at[:, c], wsems.at[k])

    def xcp(c):
        t0 = pl.multiple_of(c * T, T)
        return pltpu.make_async_copy(x_hbm.at[pl.ds(t0, T)], xin.at[pl.ds(t0, T)], xsems.at[c])

    def ocp(c):
        t0 = pl.multiple_of(c * T, T)
        return pltpu.make_async_copy(outv.at[pl.ds(t0, T)], o_hbm.at[pl.ds(t0, T)], osems.at[c])

    cp_phi = pltpu.make_async_copy(wphi_hbm, wphi_v, sems.at[0])
    cp_wo = pltpu.make_async_copy(wo_hbm, wo_v, sems.at[1])
    cp_w1 = pltpu.make_async_copy(w1_hbm, w1T, sems.at[2])
    cp_w2 = pltpu.make_async_copy(w2_hbm, w2_v, sems.at[3])

    cp_phi.start()
    wcp(1).start()
    cp_phi.wait()
    xcp(0).start()

    eye = jnp.where(lax.broadcasted_iota(i32, (H, H), 0) == lax.broadcasted_iota(i32, (H, H), 1),
                    1.0, 0.0).astype(bf16)
    for d in range(DH):
        scr[pl.ds(d, H, stride=DH), :] = _dot(eye, wphi_v[d], NT)
    for kt in range(KT):
        lo, hi = _win(kt)
        wl = hi - lo
        r = lax.broadcasted_iota(i32, (wl, DH), 0) + lo
        p = ((r.astype(f32) + 0.5) * (1.0 / PR)).astype(i32)
        et = jnp.where(((r - p * PR) >> 1) == lax.broadcasted_iota(i32, (wl, DH), 1), 1.0, 0.0).astype(bf16)
        bd = _dot(et, scr[128 * kt:128 * kt + 128, :].astype(bf16), NT)
        r2 = lax.broadcasted_iota(i32, (wl, 128), 0) + lo
        c2 = lax.broadcasted_iota(i32, (wl, 128), 1) + 128 * kt
        p2 = ((r2.astype(f32) + 0.5) * (1.0 / PR)).astype(i32)
        h2 = ((c2.astype(f32) + 0.5) * (1.0 / DH)).astype(i32)
        bdw[kt, 0:wl, :] = jnp.where((p2 * 2 + (r2 & 1)) == h2, bd, 0.0).astype(bf16)

    def fold(k, dst):
        parts = [_dot(bdw[kt, 0:_win(kt)[1] - _win(kt)[0], :],
                      wqkv_v[:, D * k + 128 * kt:D * k + 128 * (kt + 1)], NT) for kt in range(KT)]
        for b in range(0, D, 16):
            acc = _chain(jnp.add, [parts[kt][b - _win(kt)[0]:b - _win(kt)[0] + 16]
                                   for kt in range(KT) if _win(kt)[0] <= b < _win(kt)[1]])
            acc = acc - jnp.sum(acc, axis=1, keepdims=True) * (1.0 / D)
            dst[b:b + 16, :] = (acc * LOG2E).astype(bf16)

    row8 = lax.broadcasted_iota(i32, (8, T), 0)

    def put_stats(c, x):
        dT[c], r, rm = _stats(x)
        rs[c] = jnp.broadcast_to(r, (8, T))
        aux[c] = jnp.where(row8 == 0, 1.0, rm)

    def load_x(c):
        x = xin[pl.ds(pl.multiple_of(c * T, T), T), :].T
        xT[c] = x
        put_stats(c, x.astype(f32))

    def rstd_rows(c):
        return jnp.concatenate([rs[c]] * (D // 8), axis=0)

    def stage_k(c, x, r):
        pk = _dot(wkvT[0:D, :], x) * r
        for p in range(NP):
            phik[c, 2 * PR * p:2 * PR * (p + 1), :] = _phi(pk[PR * p:PR * (p + 1)])

    def stage_v(c, x, r):
        a8 = aux[c]
        vv = _dot(wkvT[D:2 * D, :], x) * r
        for p in range(NP):
            vt[c, PB * p:PB * (p + 1), :] = jnp.concatenate([vv[PR * p:PR * (p + 1)], a8], axis=0).astype(bf16)

    def stage_a(c):
        x = dT[c]
        r = rstd_rows(c)
        stage_k(c, x, r)
        stage_v(c, x, r)

    def finalize():
        r = lax.broadcasted_iota(i32, (PB, 2 * PR), 0)
        cc = lax.broadcasted_iota(i32, (PB, 2 * PR), 1)
        hsel = jnp.where(r < PR, jnp.where(r >= DH, 1, 0), jnp.where(r >= PR + 4, 1, 0))
        ok = hsel == (cc & 1)
        for p in range(NP):
            m = _chain(jnp.add, [_dot(vt[c, PB * p:PB * (p + 1), :], phik[c, 2 * PR * p:2 * PR * (p + 1), :], NT)
                                 for c in range(NC)])
            kv = m[0:PR] - csv[PR * p:PR * (p + 1), 0:2 * PR] * m[PR + 1:PR + 2]
            zz = jnp.broadcast_to(m[PR:PR + 1], (8, 2 * PR))
            kvb[p] = jnp.where(ok, jnp.concatenate([kv, zz], axis=0), 0.0).astype(bf16)

    low4 = row8 < 4

    def stage_bc(c):
        x = xT[c]
        pq = _dot(wqT[...], dT[c]) * rstd_rows(c)
        os_ = []
        for p in range(NP):
            nd = _dot(kvb[p], _phi(pq[PR * p:PR * (p + 1)]))
            rm = _rcp(nd[PR:PB] + 1e-6)
            rr = pltpu.roll(rm, 4, 0)
            ra = jnp.where(low4, rm, rr)
            rb = jnp.where(low4, rr, rm)
            os_ += [nd[0:8] * ra, nd[8:16] * ra, nd[16:24] * rm, nd[24:32] * rb, nd[32:40] * rb]
        o = jnp.concatenate(os_, axis=0).astype(bf16)
        x1 = x.astype(f32) + _dot(woT[...], o)
        hh = _dot(w1T[...], _ln(x1, 0.5))
        h = (hh + hh * jnp.tanh(hh)).astype(bf16)
        x2 = x1 + _dot(w2T[...], h)
        xb = x2.astype(bf16)
        xT[c] = xb
        put_stats(c, x2)
        outv[pl.ds(pl.multiple_of(c * T, T), T), :] = x2.T.astype(bf16)

    wcp(1).wait()
    wcp(2).start()
    fold(1, wkvT)
    xcp(0).wait()
    xcp(1).start()
    wcp(0).start()
    load_x(0)
    stage_k(0, dT[0], rstd_rows(0))
    wcp(2).wait()
    wcp(0).wait()
    xcp(1).wait()
    for c in range(2, NC):
        xcp(c).start()
    cp_wo.start()
    cp_w1.start()
    cp_w2.start()
    for j in range(KT):
        wkvT[D + 128 * j:D + 128 * (j + 1), :] = wqkv_v[:, 2 * D + 128 * j:2 * D + 128 * (j + 1)].T
    fold(0, wqT)
    stage_v(0, dT[0], rstd_rows(0))
    load_x(1)

    def body_a0(i, carry):
        @pl.when(i < NC - 1)
        def _():
            xcp(i + 1).wait()
        stage_a(i)
        load_x(jnp.minimum(i + 1, NC - 1))
        return carry
    lax.fori_loop(1, NC, body_a0, 0)

    cp_wo.wait()
    cp_w1.wait()
    cp_w2.wait()
    csv[...] = jnp.broadcast_to(jnp.sum(wkvT[D:2 * D, :].astype(f32), axis=1, keepdims=True), (D, 128))
    for j in range(KT):
        woT[128 * j:128 * (j + 1), :] = wo_v[:, 128 * j:128 * (j + 1)].T
    for j in range(F // 128):
        w2T[:, 128 * j:128 * (j + 1)] = w2_v[128 * j:128 * (j + 1), :].T
    w2T[:, F - F % 128:F] = w2_v[F - F % 128:F, :].T
    finalize()

    def layer(l, carry):
        def body_bc(i, carry):
            stage_bc(i)

            @pl.when(l == 1)
            def _():
                ocp(i).start()
            return carry
        lax.fori_loop(0, NC, body_bc, 0)

        @pl.when(l == 0)
        def _():
            def body_a(i, carry):
                stage_a(i)
                return carry
            lax.fori_loop(0, NC, body_a, 0)
            finalize()
        return carry
    lax.fori_loop(0, 2, layer, 0)
    for c in range(NC):
        ocp(c).wait()


def _make_call():
    hbm = pl.BlockSpec(memory_space=pltpu.HBM)
    return pl.pallas_call(
        _kernel,
        out_shape=jax.ShapeDtypeStruct((S, D), bf16),
        in_specs=[hbm] * 6,
        out_specs=hbm,
        scratch_shapes=[
            pltpu.VMEM((S, D), bf16),
            pltpu.VMEM((D, 3 * D), bf16),
            pltpu.VMEM((DH, DH, H), bf16),
            pltpu.VMEM((D, D), bf16),
            pltpu.VMEM((F, D), bf16),
            pltpu.VMEM((D, D), bf16),
            pltpu.VMEM((2 * D, D), bf16),
            pltpu.VMEM((D, D), bf16),
            pltpu.VMEM((F, D), bf16),
            pltpu.VMEM((D, F), bf16),
            pltpu.VMEM((NC, D, T), bf16),
            pltpu.VMEM((NC, D, T), bf16),
            pltpu.VMEM((NC, NP * 2 * PR, T), bf16),
            pltpu.VMEM((NC, NP * PB, T), bf16),
            pltpu.VMEM((NP, PB, 2 * PR), bf16),
            pltpu.VMEM((NC, 8, T), f32),
            pltpu.VMEM((NC, 8, T), f32),
            pltpu.VMEM((D, 128), f32),
            pltpu.VMEM((D, DH), f32),
            pltpu.VMEM((KT, WMAX, 128), bf16),
            pltpu.VMEM((S, D), bf16),
            pltpu.SemaphoreType.DMA((4,)),
            pltpu.SemaphoreType.DMA((3,)),
            pltpu.SemaphoreType.DMA((NC,)),
            pltpu.SemaphoreType.DMA((NC,)),
        ],
        compiler_params=pltpu.CompilerParams(vmem_limit_bytes=100 << 20),
    )


@jax.jit
def pallas_interleave_layers__linear_kernel_hedgehog__dense_activation_silu__prompt_kernel(
    A_x: jax.Array,
    A_wqkv: jax.Array,
    A_w_phi: jax.Array,
    A_wo: jax.Array,
    B_x: jax.Array,
    B_w1: jax.Array,
    B_w2: jax.Array,
):
    o = _make_call()(A_x.reshape(S, D), A_wqkv, A_w_phi.transpose(1, 2, 0), A_wo, B_w1.T, B_w2)
    return o.reshape(1, S, D)
```
